```python
import jax
import jax.numpy as jnp

def _softmax(x, axis=-1):
    return jax.nn.softmax(x, axis=axis)
def _gelu(x):
    return jax.nn.gelu(x, approximate=True)
def _silu(x):
    return jax.nn.silu(x)
def _sigmoid(x):
    return jax.nn.sigmoid(x)
def _layernorm(x, axis=-1, eps=1e-5):
    m = jnp.mean(x, axis=axis, keepdims=True)
    v = jnp.var(x, axis=axis, keepdims=True)
    return (x - m) / jnp.sqrt(v + eps)
def _scatter_add(tgt, idx, src, axis=0):
    return tgt.at[idx].add(src)
def _segment_sum(src, seg, n):
    return jax.ops.segment_sum(src, seg, n)
class _Rng:
    def __init__(self, key):
        self._k = key
    def _next(self):
        self._k, sub = jax.random.split(self._k)
        return sub
    def normal(self, shape):
        return jax.random.normal(self._next(), shape, dtype=jnp.bfloat16)
    def randint(self, lo, hi, shape):
        return jax.random.randint(self._next(), shape, lo, hi, dtype=jnp.int32)
    def uniform(self, shape, lo=0.0, hi=1.0):
        return jax.random.uniform(self._next(), shape, jnp.bfloat16, lo, hi)
    def permutation(self, n):
        return jax.random.permutation(self._next(), n)


kernel_name = 'standalone__instancenorm__prompt'

def setup_inputs():
    _rng = _Rng(jax.random.key(int.from_bytes(__import__("os").urandom(4), "little")))
    _w = (lambda a: (lambda t: t.astype(jnp.bfloat16) if jnp.issubdtype(t.dtype, jnp.floating) else t)(jnp.asarray(a)))
    B, C, H, W = 2, 1024, 2048, 32
    return {
        "x": _w((lambda *s: _rng.normal(s) * 0.05)(B, C, H, W)),
        "g": _w((lambda *s: _rng.normal(s) * 0.05)(C) + 1.0),
        "b": _w((lambda *s: _rng.normal(s) * 0.05)(C)),
    }

def reference(x, g, b):
    mu = x.mean(axis=(-2, -1), keepdims=True)
    var = ((x - mu) * (x - mu)).mean(axis=(-2, -1), keepdims=True)
    xhat = (x - mu) / jnp.sqrt(var + 1e-5)
    return xhat * g.reshape(1, -1, 1, 1) + b.reshape(1, -1, 1, 1)
```

```python
import jax
import jax.numpy as jnp
from jax import lax
import jax.experimental.pallas as pl
import jax.experimental.pallas.tpu as pltpu

_S = 8
_IPS = 8
_ROWS = 8
_CHUNKS = (1, 7, 7, 7, 7, 2, 1)
_G = 4
_CW = 512
_EPS = 1e-5


@jax.jit
def pallas_standalone__instancenorm__prompt_kernel(
    x: jax.Array,
    g: jax.Array,
    b: jax.Array,
):
    f32, bf16 = jnp.float32, jnp.bfloat16
    B, C, H, W = x.shape
    S, IPS, G, cw = _S, _IPS, _G, _CW
    RB = W // _ROWS
    K = IPS * RB
    IPB = S * IPS
    NBLK = B * C // IPB
    chunks = _CHUNKS
    assert sum(chunks) == NBLK and C % 128 == 0 and C % IPS == 0 and IPS % G == 0
    CB = max(chunks)
    starts = [sum(chunks[:i]) for i in range(len(chunks))]
    n = len(chunks)
    inv_n = 1.0 / (W * H)

    def kernel(x_hbm, g_hbm, b_hbm, o_hbm, buf, gb_v, gbf_v, gb_s, rsem, wsem, gsem):
        def rcopy(k):
            return pltpu.make_async_copy(
                x_hbm.at[pl.ds(starts[k], chunks[k])], buf.at[k % 2, pl.ds(0, chunks[k])], rsem.at[k % 2])

        def wcopy(k, t):
            a = t // K
            p = t % K
            return pltpu.make_async_copy(
                buf.at[k % 2, a, :, pl.ds(p, 1)], o_hbm.at[starts[k] + a, :, pl.ds(p, 1)], wsem.at[k % 2])

        def wwait(k):
            r = buf.at[k % 2, pl.ds(0, chunks[k])]
            pltpu.make_async_copy(r, r, wsem.at[k % 2]).wait()

        def total(acc):
            t = acc[:, :128]
            for q in range(1, cw // 128):
                t = t + acc[:, q * 128:(q + 1) * 128]
            return jnp.sum(jnp.sum(t, axis=1, keepdims=True), axis=0, keepdims=True)

        def group(k, jg):
            j0 = jg * G
            a = j0 // IPB
            s = (j0 // IPS) % S
            i0 = j0 % IPS
            ch0 = (starts[k] * IPB + j0) % C
            ref = buf.at[k % 2, a, s]

            def ld(q, r, c):
                return ref[(i0 + q) * RB + r, :, c * cw:(c + 1) * cw].astype(f32)

            means, scales = [], []
            for q in range(G):
                acc = None
                for r in range(RB):
                    for c in range(H // cw):
                        v = ld(q, r, c)
                        acc = v if acc is None else acc + v
                means.append(total(acc) * inv_n)
            for q in range(G):
                acc = None
                for r in range(RB):
                    for c in range(H // cw):
                        d = ld(q, r, c) - means[q]
                        acc = d * d if acc is None else acc + d * d
                ch = ch0 + q
                scales.append(lax.rsqrt(total(acc) * inv_n + _EPS) * gb_s[0, ch // 128, ch % 128])
            for q in range(G):
                ch = ch0 + q
                shift = gb_s[1, ch // 128, ch % 128]
                for r in range(RB):
                    for c in range(H // cw):
                        y = (ld(q, r, c) - means[q]) * scales[q] + shift
                        ref[(i0 + q) * RB + r, :, c * cw:(c + 1) * cw] = y.astype(bf16)

        def compute(k, lo, hi):
            def body(j, carry):
                group(k, j)
                return carry
            lax.fori_loop(lo, hi, body, 0)

        def write_and_compute(kw, k, ng):
            nd = chunks[kw] * K
            per = -(-nd // ng)

            def body(jj, carry):
                for p in range(per):
                    t = jj * per + p
                    if per * ng == nd:
                        wcopy(kw, t).start()
                    else:
                        @pl.when(t < nd)
                        def _():
                            wcopy(kw, t).start()
                group(k, jj)
                return carry
            lax.fori_loop(0, ng, body, 0)

        rcopy(0).start()
        cg = pltpu.make_async_copy(g_hbm, gb_v.at[0], gsem.at[0])
        cb = pltpu.make_async_copy(b_hbm, gb_v.at[1], gsem.at[1])
        cg.start()
        cb.start()
        cg.wait()
        cb.wait()
        gbf_v[...] = gb_v[...].astype(f32)
        cs = pltpu.make_async_copy(gbf_v, gb_s, gsem.at[0])
        cs.start()
        cs.wait()
        rcopy(0).wait()
        rcopy(1).start()
        compute(0, 0, chunks[0] * IPB // G)
        rcopy(1).wait()
        for k in range(1, n):
            tot = chunks[k] * IPB // G
            if k + 1 < n:
                h = tot * chunks[k - 1] // (chunks[k - 1] + chunks[k + 1])
                write_and_compute(k - 1, k, h)
                wwait(k - 1)
                rcopy(k + 1).start()
                compute(k, h, tot)
                rcopy(k + 1).wait()
            else:
                write_and_compute(k - 1, k, tot)
                wwait(k - 1)

        def last(t, carry):
            wcopy(n - 1, t).start()
            return carry
        lax.fori_loop(0, chunks[n - 1] * K, last, 0)
        wwait(n - 1)

    xt = jnp.transpose(x, (0, 1, 3, 2)).reshape(NBLK, S, K, _ROWS, H)
    y = pl.pallas_call(
        kernel,
        in_specs=[pl.BlockSpec(memory_space=pl.ANY)] * 3,
        out_specs=pl.BlockSpec(memory_space=pl.ANY),
        out_shape=jax.ShapeDtypeStruct(xt.shape, bf16),
        scratch_shapes=[
            pltpu.VMEM((2, CB, S, K, _ROWS, H), bf16),
            pltpu.VMEM((2, C // 128, 128), bf16),
            pltpu.VMEM((2, C // 128, 128), f32),
            pltpu.SMEM((2, C // 128, 128), f32),
            pltpu.SemaphoreType.DMA((2,)),
            pltpu.SemaphoreType.DMA((2,)),
            pltpu.SemaphoreType.DMA((2,)),
        ],
        compiler_params=pltpu.CompilerParams(vmem_limit_bytes=124 * 2**20),
    )(xt, g.reshape(C // 128, 128), b.reshape(C // 128, 128))
    return jnp.transpose(y.reshape(B, C, W, H), (0, 1, 3, 2))
```

```python
import jax
import jax.numpy as jnp
from jax import lax
import jax.experimental.pallas as pl
import jax.experimental.pallas.tpu as pltpu

_S = 8
_IPS = 8
_ROWS = 8
_WCOLS = 1024
_ROUNDS = (11, 11, 10)
_RWIN = 2
_G = 4
_CW = 512
_EPS = 1e-5


@jax.jit
def pallas_standalone__instancenorm__prompt_kernel(
    x: jax.Array,
    g: jax.Array,
    b: jax.Array,
):
    f32, bf16 = jnp.float32, jnp.bfloat16
    B, C, H, W = x.shape
    S, IPS, G, cw, wcols = _S, _IPS, _G, _CW, _WCOLS
    RB = W // _ROWS
    K = IPS * RB
    IPB = S * IPS
    NBLK = B * C // IPB
    NC = H // wcols
    ND = K * NC
    NG = IPB // G
    rounds = _ROUNDS
    assert sum(rounds) == NBLK and min(rounds) > _RWIN
    assert C % 128 == 0 and C % IPS == 0 and IPS % G == 0 and ND % NG == 0
    NS = max(rounds)
    starts = [sum(rounds[:i]) for i in range(len(rounds))]
    inv_n = 1.0 / (W * H)

    def kernel(x_hbm, g_hbm, b_hbm, o_hbm, buf, gb_v, gbf_v, gb_s, rsem, wsem, gsem):
        def rcopy(blk, slot):
            return pltpu.make_async_copy(x_hbm.at[blk], buf.at[slot], rsem.at[slot])

        def wstart(blk0, t):
            a = t // ND
            p = (t // NC) % K
            c = pl.multiple_of((t % NC) * wcols, wcols)
            pltpu.make_async_copy(
                buf.at[a, :, pl.ds(p, 1), :, pl.ds(c, wcols)],
                o_hbm.at[blk0 + a, :, pl.ds(p, 1), :, pl.ds(c, wcols)],
                wsem.at[0]).start()

        def wwait(nb):
            r = buf.at[pl.ds(0, nb)]
            pltpu.make_async_copy(r, r, wsem.at[0]).wait()

        def total(acc):
            t = acc[:, :128]
            for q in range(1, cw // 128):
                t = t + acc[:, q * 128:(q + 1) * 128]
            return jnp.sum(jnp.sum(t, axis=1, keepdims=True), axis=0, keepdims=True)

        def group(blk, slot, jg):
            j0 = jg * G
            s = j0 // IPS
            i0 = j0 % IPS
            ch0 = (blk * IPB + j0) % C
            ref = buf.at[slot, s]

            def ld(q, r, c):
                return ref[(i0 + q) * RB + r, :, c * cw:(c + 1) * cw].astype(f32)

            means, scales = [], []
            for q in range(G):
                acc = None
                for r in range(RB):
                    for c in range(H // cw):
                        v = ld(q, r, c)
                        acc = v if acc is None else acc + v
                means.append(total(acc) * inv_n)
            for q in range(G):
                acc = None
                for r in range(RB):
                    for c in range(H // cw):
                        d = ld(q, r, c) - means[q]
                        acc = d * d if acc is None else acc + d * d
                ch = ch0 + q
                scales.append(lax.rsqrt(total(acc) * inv_n + _EPS) * gb_s[0, ch // 128, ch % 128])
            for q in range(G):
                ch = ch0 + q
                shift = gb_s[1, ch // 128, ch % 128]
                for r in range(RB):
                    for c in range(H // cw):
                        y = (ld(q, r, c) - means[q]) * scales[q] + shift
                        ref[(i0 + q) * RB + r, :, c * cw:(c + 1) * cw] = y.astype(bf16)

        for ri, nb in enumerate(rounds):
            b0 = starts[ri]
            for j in range(_RWIN):
                rcopy(b0 + j, j).start()
            if ri == 0:
                cg = pltpu.make_async_copy(g_hbm, gb_v.at[0], gsem.at[0])
                cb = pltpu.make_async_copy(b_hbm, gb_v.at[1], gsem.at[1])
                cg.start()
                cb.start()
                cg.wait()
                cb.wait()
                gbf_v[...] = gb_v[...].astype(f32)
                cs = pltpu.make_async_copy(gbf_v, gb_s, gsem.at[0])
                cs.start()
                cs.wait()

            def block_body(j, carry, b0=b0, nb=nb):
                rcopy(b0 + j, j).wait()

                @pl.when(j + _RWIN < nb)
                def _():
                    rcopy(b0 + j + _RWIN, j + _RWIN).start()

                def body(jg, c):
                    group(b0 + j, j, jg)
                    return c
                lax.fori_loop(0, NG, body, 0)
                return carry
            lax.fori_loop(0, nb - 1, block_body, 0)

            rcopy(b0 + nb - 1, nb - 1).wait()
            per = 2 * ND // NG

            def tail_body(jg, carry, b0=b0, nb=nb):
                for p in range(per):
                    wstart(b0, jg * per + p)
                group(b0 + nb - 1, nb - 1, jg)
                return carry
            lax.fori_loop(0, NG, tail_body, 0)

            def w_body(t, carry, b0=b0):
                wstart(b0, 2 * t)
                wstart(b0, 2 * t + 1)
                return carry
            lax.fori_loop(NG * per // 2, nb * ND // 2, w_body, 0)
            wwait(nb)

    xt = jnp.transpose(x, (0, 1, 3, 2)).reshape(NBLK, S, K, _ROWS, H)
    y = pl.pallas_call(
        kernel,
        in_specs=[pl.BlockSpec(memory_space=pl.ANY)] * 3,
        out_specs=pl.BlockSpec(memory_space=pl.ANY),
        out_shape=jax.ShapeDtypeStruct(xt.shape, bf16),
        scratch_shapes=[
            pltpu.VMEM((NS, S, K, _ROWS, H), bf16),
            pltpu.VMEM((2, C // 128, 128), bf16),
            pltpu.VMEM((2, C // 128, 128), f32),
            pltpu.SMEM((2, C // 128, 128), f32),
            pltpu.SemaphoreType.DMA((NS,)),
            pltpu.SemaphoreType.DMA((1,)),
            pltpu.SemaphoreType.DMA((2,)),
        ],
        compiler_params=pltpu.CompilerParams(vmem_limit_bytes=120 * 2**20),
    )(xt, g.reshape(C // 128, 128), b.reshape(C // 128, 128))
    return jnp.transpose(y.reshape(B, C, W, H), (0, 1, 3, 2))
```

```python
import jax
import jax.numpy as jnp
from jax import lax
import jax.experimental.pallas as pl
import jax.experimental.pallas.tpu as pltpu

_S = 8
_IPS = 8
_ROWS = 8
_WCOLS = 1024
_ROUNDS = (11, 11, 10)
_RWIN = 2
_WPRE = 2
_G = 4
_CW = 512
_EPS = 1e-5


@jax.jit
def pallas_standalone__instancenorm__prompt_kernel(
    x: jax.Array,
    g: jax.Array,
    b: jax.Array,
):
    f32, bf16 = jnp.float32, jnp.bfloat16
    B, C, H, W = x.shape
    S, IPS, G, cw, wcols = _S, _IPS, _G, _CW, _WCOLS
    RB = W // _ROWS
    K = IPS * RB
    IPB = S * IPS
    NBLK = B * C // IPB
    NC = H // wcols
    ND = K * NC
    NG = IPB // G
    rounds = _ROUNDS
    assert sum(rounds) == NBLK and min(rounds) > max(_RWIN, 3) and _WPRE % 2 == 0
    assert C % 128 == 0 and C % IPS == 0 and IPS % G == 0 and ND % NG == 0
    NS = max(rounds)
    starts = [sum(rounds[:i]) for i in range(len(rounds))]
    inv_n = 1.0 / (W * H)

    def kernel(x_hbm, g_hbm, b_hbm, o_hbm, buf, gb_v, gbf_v, gb_s, rsem, wsem, gsem):
        def rcopy(blk, slot):
            return pltpu.make_async_copy(x_hbm.at[blk], buf.at[slot], rsem.at[slot])

        def rlast(blk, slot):
            h = K // 2 + 1
            return (pltpu.make_async_copy(x_hbm.at[blk, :, pl.ds(0, h)], buf.at[slot, :, pl.ds(0, h)],
                                          rsem.at[slot]),
                    pltpu.make_async_copy(x_hbm.at[blk, :, pl.ds(h, K - h)], buf.at[slot, :, pl.ds(h, K - h)],
                                          rsem.at[NS]))

        def wstart(blk0, t):
            a = t // ND
            p = (t // NC) % K
            c = pl.multiple_of((t % NC) * wcols, wcols)
            pltpu.make_async_copy(
                buf.at[a, :, pl.ds(p, 1), :, pl.ds(c, wcols)],
                o_hbm.at[blk0 + a, :, pl.ds(p, 1), :, pl.ds(c, wcols)],
                wsem.at[0]).start()

        def wwait(nb):
            r = buf.at[pl.ds(0, nb)]
            pltpu.make_async_copy(r, r, wsem.at[0]).wait()

        def total(acc):
            t = acc[:, :128]
            for q in range(1, cw // 128):
                t = t + acc[:, q * 128:(q + 1) * 128]
            return jnp.sum(jnp.sum(t, axis=1, keepdims=True), axis=0, keepdims=True)

        def group(blk, slot, jg):
            j0 = jg * G
            s = j0 // IPS
            i0 = j0 % IPS
            ch0 = (blk * IPB + j0) % C
            ref = buf.at[slot, s]

            def ld(q, r, c):
                return ref[(i0 + q) * RB + r, :, c * cw:(c + 1) * cw].astype(f32)

            means, scales = [], []
            for q in range(G):
                acc = None
                for r in range(RB):
                    for c in range(H // cw):
                        v = ld(q, r, c)
                        acc = v if acc is None else acc + v
                means.append(total(acc) * inv_n)
            for q in range(G):
                acc = None
                for r in range(RB):
                    for c in range(H // cw):
                        d = ld(q, r, c) - means[q]
                        acc = d * d if acc is None else acc + d * d
                ch = ch0 + q
                scales.append(lax.rsqrt(total(acc) * inv_n + _EPS) * gb_s[0, ch // 128, ch % 128])
            for q in range(G):
                ch = ch0 + q
                shift = gb_s[1, ch // 128, ch % 128]
                for r in range(RB):
                    for c in range(H // cw):
                        y = (ld(q, r, c) - means[q]) * scales[q] + shift
                        ref[(i0 + q) * RB + r, :, c * cw:(c + 1) * cw] = y.astype(bf16)

        for ri, nb in enumerate(rounds):
            b0 = starts[ri]
            for j in range(_RWIN):
                rcopy(b0 + j, j).start()
            if ri == 0:
                cg = pltpu.make_async_copy(g_hbm, gb_v.at[0], gsem.at[0])
                cb = pltpu.make_async_copy(b_hbm, gb_v.at[1], gsem.at[1])
                cg.start()
                cb.start()
                cg.wait()
                cb.wait()
                gbf_v[...] = gb_v[...].astype(f32)
                cs = pltpu.make_async_copy(gbf_v, gb_s, gsem.at[0])
                cs.start()
                cs.wait()

            def block_body(j, carry, b0=b0, nb=nb):
                rcopy(b0 + j, j).wait()

                @pl.when(j + _RWIN < nb - 1)
                def _():
                    rcopy(b0 + j + _RWIN, j + _RWIN).start()

                @pl.when(j + _RWIN == nb - 1)
                def _():
                    for c in rlast(b0 + nb - 1, nb - 1):
                        c.start()

                def body(jg, c):
                    group(b0 + j, j, jg)
                    return c
                lax.fori_loop(0, NG, body, 0)
                return carry
            lax.fori_loop(0, nb - 1, block_body, 0)

            big, small = rlast(b0 + nb - 1, nb - 1)
            small.wait()
            for p in range(_WPRE):
                wstart(b0, p)
            big.wait()
            per = 2 * ND // NG

            def tail_body(jg, carry, b0=b0, nb=nb):
                for p in range(per):
                    wstart(b0, _WPRE + jg * per + p)
                group(b0 + nb - 1, nb - 1, jg)
                return carry
            lax.fori_loop(0, NG, tail_body, 0)

            def w_body(t, carry, b0=b0):
                wstart(b0, 2 * t)
                wstart(b0, 2 * t + 1)
                return carry
            lax.fori_loop((_WPRE + NG * per) // 2, nb * ND // 2, w_body, 0)
            wwait(nb)

    xt = jnp.transpose(x, (0, 1, 3, 2)).reshape(NBLK, S, K, _ROWS, H)
    y = pl.pallas_call(
        kernel,
        in_specs=[pl.BlockSpec(memory_space=pl.ANY)] * 3,
        out_specs=pl.BlockSpec(memory_space=pl.ANY),
        out_shape=jax.ShapeDtypeStruct(xt.shape, bf16),
        scratch_shapes=[
            pltpu.VMEM((NS, S, K, _ROWS, H), bf16),
            pltpu.VMEM((2, C // 128, 128), bf16),
            pltpu.VMEM((2, C // 128, 128), f32),
            pltpu.SMEM((2, C // 128, 128), f32),
            pltpu.SemaphoreType.DMA((NS + 1,)),
            pltpu.SemaphoreType.DMA((1,)),
            pltpu.SemaphoreType.DMA((2,)),
        ],
        compiler_params=pltpu.CompilerParams(vmem_limit_bytes=120 * 2**20),
    )(xt, g.reshape(C // 128, 128), b.reshape(C // 128, 128))
    return jnp.transpose(y.reshape(B, C, W, H), (0, 1, 3, 2))
```
